```python
import jax
import jax.numpy as jnp

def _softmax(x, axis=-1):
    return jax.nn.softmax(x, axis=axis)
def _gelu(x):
    return jax.nn.gelu(x, approximate=True)
def _silu(x):
    return jax.nn.silu(x)
def _sigmoid(x):
    return jax.nn.sigmoid(x)
def _layernorm(x, axis=-1, eps=1e-5):
    m = jnp.mean(x, axis=axis, keepdims=True)
    v = jnp.var(x, axis=axis, keepdims=True)
    return (x - m) / jnp.sqrt(v + eps)
def _scatter_add(tgt, idx, src, axis=0):
    return tgt.at[idx].add(src)
def _segment_sum(src, seg, n):
    return jax.ops.segment_sum(src, seg, n)
class _Rng:
    def __init__(self, key):
        self._k = key
    def _next(self):
        self._k, sub = jax.random.split(self._k)
        return sub
    def normal(self, shape):
        return jax.random.normal(self._next(), shape, dtype=jnp.bfloat16)
    def randint(self, lo, hi, shape):
        return jax.random.randint(self._next(), shape, lo, hi, dtype=jnp.int32)
    def uniform(self, shape, lo=0.0, hi=1.0):
        return jax.random.uniform(self._next(), shape, jnp.bfloat16, lo, hi)
    def permutation(self, n):
        return jax.random.permutation(self._next(), n)


kernel_name = 'standalone__self_sup_conv_stem_wavlm__speech'

def setup_inputs():
    _rng = _Rng(jax.random.key(int.from_bytes(__import__("os").urandom(4), "little")))
    _w = (lambda a: (lambda t: t.astype(jnp.bfloat16) if jnp.issubdtype(t.dtype, jnp.floating) else t)(jnp.asarray(a)))
    B, T, D, K = 2, 16000, 512, 31
    scale = (K * D) ** -0.5
    return {
        "x": _w((lambda *s: _rng.normal(s) * 0.05)(B, T, D)),
        "w": _w((lambda *s: _rng.normal(s) * 0.05)(K, D, D) * scale),
        "gn_gamma": _w((lambda *s: _rng.normal(s) * 0.05)(D) * 0.1 + 1.0),
        "gn_beta": _w((lambda *s: _rng.normal(s) * 0.05)(D) * 0.1),
    }

def reference(x, w, gn_gamma, gn_beta):
    B, T, D = x.shape
    K = w.shape[0]
    s = 2
    L = (T - K) // s + 1
    h = jnp.einsum('blc,cd->bld', x[:, 0:s * L:s, :], w[0])
    for i in range(1, K):
        h = h + jnp.einsum('blc,cd->bld', x[:, i:i + s * L:s, :], w[i])
    mu = jnp.einsum('bld->bd', h)[:, None, :] / L
    var = jnp.einsum('bld->bd', (h - mu) ** 2)[:, None, :] / L
    h = (h - mu) / jnp.sqrt(var + 1e-5)
    h = h * gn_gamma[None, None, :] + gn_beta[None, None, :]
    return _gelu(h)
```

```python
import jax
import jax.numpy as jnp
import jax.experimental.pallas as pl
import jax.experimental.pallas.tpu as pltpu


def _gelu(h):
    c = 0.7978845608028654
    inner = c * (h + 0.044715 * (h * h * h))
    return 0.5 * h * (1.0 + jnp.tanh(inner))


@jax.jit
def pallas_standalone__self_sup_conv_stem_wavlm__speech_kernel(
    x: jax.Array,
    w: jax.Array,
    gn_gamma: jax.Array,
    gn_beta: jax.Array,
):
    B, T, D = x.shape
    K = w.shape[0]
    L = (T - K) // 2 + 1
    TM = 512
    NCH = (L + TM - 1) // TM
    LP = NCH * TM
    H2 = T // 2

    def kernel(x_ref, w_ref, g_ref, b_ref, o_ref, xp_ref, h_ref):
        zpad = jnp.zeros((LP + 16 - H2, 2 * D), jnp.bfloat16)
        xp_ref[H2:, :] = zpad

        def split(i, c):
            r0 = pl.multiple_of(i * 500, 4)
            return c

        for i in range(H2 // 320):
            u = pltpu.bitcast(x_ref[0, i * 640:(i + 1) * 640, :], jnp.uint32)
            e = pltpu.bitcast(u << 16, jnp.float32).astype(jnp.bfloat16)
            o = pltpu.bitcast(u & jnp.uint32(0xFFFF0000), jnp.float32).astype(jnp.bfloat16)
            xp_ref[i * 320:(i + 1) * 320, :D] = e
            xp_ref[i * 320:(i + 1) * 320, D:] = o

        def chunk(i, carry):
            s1, s2 = carry
            r0 = pl.multiple_of(i * TM, TM)
            xs = xp_ref[pl.ds(r0, TM + 16), :]
            acc = jnp.zeros((TM, D), jnp.float32)
            for j in range(16):
                xj = xs[j:j + TM, :]
                acc = acc + jnp.dot(xj[:, :D], w_ref[2 * j], preferred_element_type=jnp.float32)
                if 2 * j + 1 < K:
                    acc = acc + jnp.dot(xj[:, D:], w_ref[2 * j + 1], preferred_element_type=jnp.float32)
            rows = r0 + jax.lax.broadcasted_iota(jnp.int32, (TM, D), 0)
            acc = jnp.where(rows < L, acc, 0.0)
            h_ref[pl.ds(r0, TM), :] = acc
            s1 = s1 + jnp.sum(acc, axis=0, keepdims=True)
            return s1, s2

        z = jnp.zeros((1, D), jnp.float32)
        s1, _ = jax.lax.fori_loop(0, NCH, chunk, (z, z))
        mu = s1 / L

        def var_chunk(i, s2):
            r0 = pl.multiple_of(i * TM, TM)
            hh = h_ref[pl.ds(r0, TM), :]
            rows = r0 + jax.lax.broadcasted_iota(jnp.int32, (TM, D), 0)
            d = jnp.where(rows < L, hh - mu, 0.0)
            return s2 + jnp.sum(d * d, axis=0, keepdims=True)

        s2 = jax.lax.fori_loop(0, NCH, var_chunk, z)
        rstd = jax.lax.rsqrt(s2 / L + 1e-5)
        sc = rstd * g_ref[...].astype(jnp.float32)
        sh = b_ref[...].astype(jnp.float32) - mu * sc

        nfull = L // TM

        def out_chunk(i, c):
            r0 = pl.multiple_of(i * TM, TM)
            hh = h_ref[pl.ds(r0, TM), :]
            o_ref[0, pl.ds(r0, TM), :] = _gelu(hh * sc + sh).astype(o_ref.dtype)
            return c

        jax.lax.fori_loop(0, nfull, out_chunk, 0)
        rem = L - nfull * TM
        hh = h_ref[nfull * TM:nfull * TM + rem, :]
        o_ref[0, nfull * TM:, :] = _gelu(hh * sc + sh).astype(o_ref.dtype)

    return pl.pallas_call(
        kernel,
        grid=(B,),
        in_specs=[
            pl.BlockSpec((1, T, D), lambda b: (b, 0, 0)),
            pl.BlockSpec((K, D, D), lambda b: (0, 0, 0), pipeline_mode=pl.Buffered(1)),
            pl.BlockSpec((1, D), lambda b: (0, 0)),
            pl.BlockSpec((1, D), lambda b: (0, 0)),
        ],
        out_specs=pl.BlockSpec((1, L, D), lambda b: (b, 0, 0)),
        out_shape=jax.ShapeDtypeStruct((B, L, D), x.dtype),
        scratch_shapes=[
            pltpu.VMEM((LP + 16, 2 * D), jnp.bfloat16),
            pltpu.VMEM((LP, D), jnp.float32),
        ],
        compiler_params=pltpu.CompilerParams(
            dimension_semantics=("arbitrary",),
            vmem_limit_bytes=120 * 1024 * 1024,
        ),
    )(x, w, gn_gamma.reshape(1, D), gn_beta.reshape(1, D))
```

```python
import math
import numpy as np
import jax
import jax.numpy as jnp
import jax.experimental.pallas as pl
import jax.experimental.pallas.tpu as pltpu

N = 40
M = 25
C1 = math.cos(2 * math.pi / 5); C2 = math.cos(4 * math.pi / 5)
S1 = math.sin(2 * math.pi / 5); S2 = math.sin(4 * math.pi / 5)
R2 = math.sqrt(0.5)


class V:
    __slots__ = ("val", "neg")

    def __init__(self, val, neg=False):
        self.val = val
        self.neg = neg

    def get(self):
        return -self.val if self.neg else self.val


ZERO = V(None)


def vneg(a):
    return V(a.val, not a.neg)


def vadd(a, b):
    if a.val is None:
        return b
    if b.val is None:
        return a
    if a.neg == b.neg:
        return V(a.val + b.val, a.neg)
    if b.neg:
        return V(a.val - b.val, False)
    return V(b.val - a.val, False)


def vsub(a, b):
    return vadd(a, vneg(b))


def vmul(c, a):
    if a.val is None:
        return a
    return V(a.val * np.float32(-c if a.neg else c), False)


def cadd(a, b): return (vadd(a[0], b[0]), vadd(a[1], b[1]))
def csub(a, b): return (vsub(a[0], b[0]), vsub(a[1], b[1]))
def cmulr(c, a): return (vmul(c, a[0]), vmul(c, a[1]))


def cadd_i(a, b, s):
    if s > 0:
        return (vsub(a[0], b[1]), vadd(a[1], b[0]))
    return (vadd(a[0], b[1]), vsub(a[1], b[0]))


def dft5(x, s):
    t1 = cadd(x[1], x[4]); t2 = cadd(x[2], x[3]); t3 = csub(x[1], x[4]); t4 = csub(x[2], x[3])
    t5 = cadd(t1, t2)
    X0 = cadd(x[0], t5)
    a0 = cadd(x[0], cmulr((C1 + C2) / 2, t5))
    m2 = cmulr((C1 - C2) / 2, csub(t1, t2))
    a1 = cadd(a0, m2); a2 = csub(a0, m2)
    b1 = cadd(cmulr(S1, t3), cmulr(S2, t4))
    b2 = csub(cmulr(S2, t3), cmulr(S1, t4))
    return [X0, cadd_i(a1, b1, s), cadd_i(a2, b2, s), cadd_i(a2, b2, -s), cadd_i(a1, b1, -s)]


def dft4(x, s):
    a = cadd(x[0], x[2]); b = csub(x[0], x[2]); c = cadd(x[1], x[3]); d = csub(x[1], x[3])
    return [cadd(a, c), cadd_i(b, d, s), csub(a, c), cadd_i(b, d, -s)]


def dft8(x, s):
    E = dft4(x[0::2], s); O = dft4(x[1::2], s)
    o1 = O[1]; o3 = O[3]
    if s > 0:
        t1 = (vmul(R2, vsub(o1[0], o1[1])), vmul(R2, vadd(o1[0], o1[1])))
        t3 = (vmul(-R2, vadd(o3[0], o3[1])), vmul(R2, vsub(o3[0], o3[1])))
    else:
        t1 = (vmul(R2, vadd(o1[0], o1[1])), vmul(R2, vsub(o1[1], o1[0])))
        t3 = (vmul(R2, vsub(o3[1], o3[0])), vmul(-R2, vadd(o3[0], o3[1])))
    out = [None] * 8
    out[0] = cadd(E[0], O[0]); out[4] = csub(E[0], O[0])
    out[1] = cadd(E[1], t1); out[5] = csub(E[1], t1)
    out[2] = cadd_i(E[2], O[2], s); out[6] = cadd_i(E[2], O[2], -s)
    out[3] = cadd(E[3], t3); out[7] = csub(E[3], t3)
    return out


def crt(k1, k2):
    return [k for k in range(N) if k % 5 == k1 and k % 8 == k2][0]


def _gelu(h):
    c = 0.7978845608028654
    inner = h * (np.float32(c) + np.float32(c * 0.044715) * (h * h))
    return (np.float32(0.5) * h) * (np.float32(1.0) + jnp.tanh(inner))


def _gelu_half(u):
    c = 0.7978845608028654
    z = u * (np.float32(2 * c) + np.float32(8 * c * 0.044715) * (u * u))
    return u + u * jnp.tanh(z)


@jax.jit
def pallas_standalone__self_sup_conv_stem_wavlm__speech_kernel(
    x: jax.Array,
    w: jax.Array,
    gn_gamma: jax.Array,
    gn_beta: jax.Array,
):
    B, T, D = x.shape
    K = w.shape[0]
    L = (T - K) // 2 + 1
    assert (B, T, D, K) == (2, 16000, 512, 31)
    U = T // 2
    G = 5
    TC = 2 * 8 * G
    NCH = U // (M * 8 * G)
    CU = M * 8 * G
    XR = 2032
    XB = 2064
    NI = 20
    OB = 2048
    HROWS = 8 * U
    UNROLL = 2
    KSPLIT = 2
    FFT_WEIGHT = 16 * 54 + 5 * 152
    NG = 1

    def kernel(flag_ref, x_hbm, w_hbm, g_ref, b_ref, o_hbm, wh0, wh1, wh2, wh3, xh0, xh1, yh0, yh1, xs, hb, st, tF0, tF1, tI0, tI1, xsem, wsem, osem):
        whs = [wh0, wh1, wh2, wh3]
        tF = [tF0, tF1]
        tI = [tI0, tI1]
        dz = flag_ref[0]
        dz2 = flag_ref[1]
        xh = [xh0, xh1]
        yh = [yh0, yh1]
        xs32 = xs
        hb32 = hb
        xs = xs32.bitcast(jnp.bfloat16)
        hb = hb32.bitcast(jnp.bfloat16)
        hmask = np.uint32(0xFFFF0000)

        def x_copies(c, slot, dts=(0, 1, 2, 3)):
            start = pl.multiple_of(jnp.minimum(c * (2 * CU), T - XR), 16)
            return [pltpu.make_async_copy(
                x_hbm.at[b, pl.ds(start, XR), pl.ds(128 * dt, 128)],
                xs.at[pl.ds(pl.multiple_of(((slot * 2 + b) * 4 + dt) * XB, 16), XR), :], xsem.at[slot * 4 + dt])
                for dt in dts for b in range(2)]

        def w_copies(dt):
            return [pltpu.make_async_copy(
                w_hbm.at[:, pl.ds(128 * dt, 128)],
                hb.at[pl.ds(dt * K * D, K * D), :], wsem.at[dt])]

        for cp in x_copies(0, 0):
            cp.start()

        for i in range(16):
            xs32[(i * XB + XR) // 2:(i + 1) * XB // 2, :] = jnp.zeros(((XB - XR) // 2, 128), jnp.uint32)
        for slot in range(2):
            xh[slot][0] = jnp.zeros((TC // 2, 2 * D), jnp.uint32)
        st[...] = jnp.zeros(st.shape, jnp.float32)

        TOK = [None]
        never_s = [flag_ref[0] > 0]

        def gate(v):
            if TOK[0] is None:
                return v
            t = TOK[0]
            if v.dtype != t.dtype:
                t = pltpu.bitcast(t, v.dtype)
            return jnp.where(never_s[0], t, v)

        def gateV(a):
            return V(gate(a.val), a.neg)

        def stash(ref, idx, cv):
            out = []
            for c_, v in enumerate(cv):
                if v.val is None:
                    out.append(None)
                else:
                    ref[dz + 2 * idx + c_] = v.val
                    out.append(v.neg)
            return out

        def fetch(ref, idx, negs):
            return tuple(ZERO if ng is None else V(ref[dz2 + 2 * idx + c_], ng) for c_, ng in enumerate(negs))

        def fft_unit(slot, off, g, dt, tr=0):
            base = (slot * 8 + dt) * (XB // 2) + off + g * (8 * M)
            lane0 = pl.multiple_of(dt * 128, 128)
            lane1 = pl.multiple_of(dt * 128 + D, 128)
            row0 = pl.multiple_of(g * 8, 8)
            T1 = []
            for b in range(2):
                Tb = []
                for p2 in range(8):
                    zin = []
                    for p1 in range(5):
                        p = (8 * p1 + 5 * p2) % N
                        u = xs32[pl.ds(base + b * (2 * XB) + p, 8, stride=M), :]
                        if p1 < NG:
                            u = gate(u)
                        zin.append((V(pltpu.bitcast(u << 16, jnp.float32)),
                                    V(pltpu.bitcast(u & hmask, jnp.float32))))
                    o5 = dft5(zin, -1)
                    Tb.append([stash(tF[tr], (b * 8 + p2) * 5 + k1, o5[k1]) for k1 in range(5)])
                    yield 54
                T1.append(Tb)

            def emit(m, lane, va, vb):
                v = pltpu.pack_elementwise([va.get(), vb.get()], packed_dtype=jnp.bfloat16)
                xh[slot][m, pl.ds(row0, 8), pl.ds(lane, 128)] = pltpu.bitcast(v, jnp.uint32)

            for k1 in range(5):
                r = []
                for b in range(2):
                    zz = [fetch(tF[tr], (b * 8 + p2) * 5 + k1, T1[b][p2][k1]) for p2 in range(8)]
                    zz[0] = (gateV(zz[0][0]), zz[0][1])
                    r.append(dft8(zz, -1))
                    yield 56
                for k2 in range(8):
                    k = crt(k1, k2)
                    (a0, b0), (a1, b1) = r[0][k2], r[1][k2]
                    if k == 0:
                        emit(2, lane0, a0, a1); emit(2, lane1, b0, b1)
                    elif k == 20:
                        emit(1, lane0, a0, a1); emit(1, lane1, b0, b1)
                    elif k < 20:
                        emit(3 * k, lane0, vadd(a0, b0), vadd(a1, b1))
                        emit(3 * k + 1, lane0, a0, a1)
                        emit(3 * k + 2, lane0, b0, b1)
                    else:
                        kk = N - k
                        emit(3 * kk, lane1, vsub(a0, b0), vsub(a1, b1))
                        emit(3 * kk + 1, lane1, a0, a1)
                        emit(3 * kk + 2, lane1, b0, b1)
                yield 40

        def w_unit(dt, rb, tr=0):
            T1 = []
            raw = {}

            def getraw(j):
                if j not in raw:
                    raw[j] = hb32[pl.ds(pl.multiple_of((dt * K + j) * (D // 2) + rb * 8, 8), 8), :]
                return raw[j]
            for h in range(2):
                def ld(j, gt=False):
                    if j >= K:
                        return ZERO
                    u = getraw(j)
                    if gt:
                        u = gate(u)
                    return V(pltpu.bitcast((u << 16) if h == 0 else (u & hmask), jnp.float32))
                Tb = []
                for p2 in range(8):
                    zin = []
                    first = True
                    for p1 in range(5):
                        p = (8 * p1 + 5 * p2) % N
                        if p < 16:
                            zin.append((ld(2 * p, first), vneg(ld(2 * p + 1))))
                            first = False
                        else:
                            zin.append((ZERO, ZERO))
                    o5 = dft5(zin, +1)
                    Tb.append([stash(tF[tr], (h * 8 + p2) * 5 + k1, o5[k1]) for k1 in range(5)])
                    yield 32
                T1.append(Tb)

            def emit(m, half, va, vb):
                v = pltpu.pack_elementwise([va.get(), vb.get()], packed_dtype=jnp.bfloat16)
                whs[dt][m, pl.ds(pl.multiple_of(half * (D // 2) + rb * 8, 8), 8), :] = pltpu.bitcast(v, jnp.uint32)

            for k1 in range(5):
                r = []
                for h in range(2):
                    zz = [fetch(tF[tr], (h * 8 + p2) * 5 + k1, T1[h][p2][k1]) for p2 in range(8)]
                    zz[0] = (gateV(zz[0][0]), zz[0][1])
                    r.append(dft8(zz, +1))
                    yield 56
                for k2 in range(8):
                    k = crt(k1, k2)
                    q = [r[0][k2], r[1][k2]]
                    if k == 0:
                        emit(2, 0, *[vmul(-2.0, a[0]) for a in q])
                        emit(2, 1, *[vmul(2.0, a[1]) for a in q])
                    elif k == 20:
                        emit(1, 0, *[vmul(2.0, a[0]) for a in q])
                        emit(1, 1, *[vmul(-2.0, a[1]) for a in q])
                    elif k < 20:
                        emit(3 * k, 0, *[a[0] for a in q])
                        emit(3 * k + 1, 0, *[vsub(a[1], a[0]) for a in q])
                        emit(3 * k + 2, 0, *[vadd(a[0], a[1]) for a in q])
                    else:
                        kk = N - k
                        emit(3 * kk, 1, *[a[0] for a in q])
                        emit(3 * kk + 1, 1, *[vneg(vadd(a[0], a[1])) for a in q])
                        emit(3 * kk + 2, 1, *[vsub(a[1], a[0]) for a in q])
                yield 66
        W_WEIGHT = 16 * 32 + 5 * (112 + 66)

        def chain(gens):
            for g_ in gens:
                yield from g_

        def mm_piece(slot, kap, dt):
            ks = []
            for j in range(3):
                acc = None
                for kh in range(KSPLIT):
                    kw = 2 * D // KSPLIT
                    a = pltpu.bitcast(xh[slot][3 * kap + j, :, kh * kw:(kh + 1) * kw], jnp.bfloat16)
                    mw = jnp.maximum(3 * kap, 1) if j == 0 else 3 * kap + j
                    bb = pltpu.bitcast(whs[dt][mw, kh * kw // 2:(kh + 1) * kw // 2, :], jnp.bfloat16)
                    d = jnp.dot(a, bb, preferred_element_type=jnp.float32)
                    acc = d if acc is None else acc + d
                    TOK[0] = d[0:8, :]
                    yield 1
                ks.append(acc)
            r0 = pl.multiple_of((2 * kap * 4 + dt) * TC, 8)
            r1 = pl.multiple_of(((2 * kap + 1) * 4 + dt) * TC, 8)
            yh[slot][pl.ds(r0, TC), :] = ks[0] - ks[2]
            yh[slot][pl.ds(r1, TC), :] = ks[0] + ks[1]

        def mm_unit(slot, kap):
            for dt in range(4):
                yield from mm_piece(slot, kap, dt)

        def run_all(gen):
            for _ in gen:
                pass

        def interleave(mm, others, npieces):
            tot = sum(w for _, w in others)
            done = [0.0] * len(others)
            alive = [True] * len(others)
            i = 0
            for _ in mm:
                i += 1
                target = tot * min(i, npieces) / npieces
                while sum(done) < target and any(alive):
                    k = min((k for k in range(len(others)) if alive[k]), key=lambda k: done[k] / others[k][1])
                    try:
                        done[k] += next(others[k][0])
                    except StopIteration:
                        alive[k] = False
            for gen, _ in others:
                run_all(gen)

        def ifft_unit(slot, c, g, dt, masked, tr=0):
            rowa = dt * TC + g * 16
            rowb = rowa + 1

            def ld(v, row):
                return V(yh[slot][pl.ds(v * (4 * TC) + row, 8, stride=2), :])
            Dk = [None] * N
            Dk[0] = (ld(0, rowa), ld(0, rowb))
            Dk[20] = (ld(1, rowa), ld(1, rowb))
            for k in range(1, 20):
                ar, ai = ld(2 * k, rowa), ld(2 * k + 1, rowa)
                br, bi = ld(2 * k, rowb), ld(2 * k + 1, rowb)
                Dk[k] = (vsub(ar, bi), vadd(ai, br))
                Dk[N - k] = (vadd(ar, bi), vsub(br, ai))
            T1 = [None] * 8
            for p2 in (0, 1, 7, 2, 6, 3, 5, 4):
                o5 = dft5([(gateV(Dk[(8 * p1 + 5 * p2) % N][0]), Dk[(8 * p1 + 5 * p2) % N][1]) if p1 < NG else Dk[(8 * p1 + 5 * p2) % N] for p1 in range(5)], +1)
                T1[p2] = [stash(tI[tr], p2 * 5 + k1, o5[k1]) for k1 in range(5)]
                yield 54
            t0 = c * (8 * G) + g * 8
            hrow = t0 * (4 * M) + dt
            s = [None] * 4
            if masked:
                lrow = (t0 + jax.lax.broadcasted_iota(jnp.int32, (8, 128), 0)) * M
            for k1 in range(5):
                zz = [fetch(tI[tr], p2 * 5 + k1, T1[p2][k1]) for p2 in range(8)]
                zz[0] = (gateV(zz[0][0]), zz[0][1])
                r = dft8(zz, +1)
                for k2 in range(8):
                    n = crt(k1, k2)
                    if n >= M:
                        continue
                    h0, h1 = r[k2][0].get(), r[k2][1].get()
                    if masked:
                        ok = lrow < (L - n)
                        h0 = jnp.where(ok, h0, 0.0)
                        h1 = jnp.where(ok, h1, 0.0)
                    for i, hv in enumerate((h0, h1)):
                        sq = hv * hv
                        s[2 * i] = hv if s[2 * i] is None else s[2 * i] + hv
                        s[2 * i + 1] = sq if s[2 * i + 1] is None else s[2 * i + 1] + sq
                    pk = pltpu.pack_elementwise([h0, h1], packed_dtype=jnp.bfloat16)
                    hb32[pl.ds(hrow + 4 * n, 8, stride=4 * M), :] = pltpu.bitcast(pk, jnp.uint32)
                yield 90
            for i in range(4):
                idx = dt * 4 + i
                st[idx] = st[idx] + s[i]

        def pro_body(i, carry):
            dt = i // G

            @pl.when(i % G == 0)
            def _():
                for b in range(2):
                    pltpu.make_async_copy(
                        x_hbm.at[b, pl.ds(0, XR), pl.ds(0, 128)],
                        xs.at[pl.ds(0, XR), :], xsem.at[dt]).wait()

            @pl.when(i == G)
            def _():
                for cp in w_copies(0):
                    cp.start()

            @pl.when(i == 3 * G)
            def _():
                for cp in w_copies(1):
                    cp.start()
                for cp in x_copies(1, 1):
                    cp.start()
            run_all(fft_unit(0, 0, i % G, dt))
            return carry
        jax.lax.fori_loop(0, NI, pro_body, 0)

        for cp in w_copies(0):
            cp.wait()

        def w_body(rb, carry):
            run_all(w_unit(0, rb))
            return carry
        jax.lax.fori_loop(0, D // 16, w_body, 0)

        def stage(dt):
            for cp in w_copies(dt + 1):
                cp.wait()
            if dt + 2 < 4:
                for cp in w_copies(dt + 2):
                    cp.start()

            def body(it, carry):
                mm = chain([mm_piece(0, it * 5 + u, dt) for u in range(5)])
                others = [(chain([w_unit(dt + 1, it * 8 + u, u % 2) for u in range(8)]), 8 * W_WEIGHT)]
                interleave(mm, others, 15 * KSPLIT)
                TOK[0] = None
                return carry
            jax.lax.fori_loop(0, 4, body, 0)
        for dt_ in range(3):
            stage(dt_)

        for cp in x_copies(1, 1):
            cp.wait()
        for cp in x_copies(2, 0):
            cp.start()

        def stage3_body(it, carry):
            mm = chain([mm_piece(0, it * 5 + u, 3) for u in range(5)])
            others = [(chain([fft_unit(1, 0, (it * 5 + u) // 4, (it * 5 + u) % 4, u % 2) for u in range(5)]), 5 * FFT_WEIGHT)]
            interleave(mm, others, 15 * KSPLIT)
            TOK[0] = None
            return carry
        jax.lax.fori_loop(0, 4, stage3_body, 0)

        def phase(p, cur, do_fft=True):
            nxt = 1 - cur
            if do_fft:
                for cp in x_copies(p + 1, nxt):
                    cp.wait()

                @pl.when(p + 2 < NCH)
                def _():
                    for cp in x_copies(p + 2, cur):
                        cp.start()
            off = jnp.where(p + 1 >= NCH - 1, (XR - 2 * CU) // 2, 0)
            cprev = p - 1

            def body(i, carry):
                for u in range(UNROLL):
                    ii = i * UNROLL + u
                    others = [(ifft_unit(nxt, cprev, ii // 4, ii % 4, False, u % 2), 8 * 54 + 5 * 90)]
                    if do_fft:
                        others.append((fft_unit(nxt, off, ii // 4, ii % 4, u % 2), FFT_WEIGHT))
                    interleave(mm_unit(cur, ii), others, 12 * KSPLIT)
                    TOK[0] = None
                return carry
            jax.lax.fori_loop(0, NI // UNROLL, body, 0)

        def phase2(q, carry):
            phase(2 * q + 1, 1)
            phase(2 * q + 2, 0)
            return carry
        jax.lax.fori_loop(0, NCH // 2 - 1, phase2, 0)
        phase(NCH - 1, 1, do_fft=False)
        pl_last = NCH - 1

        def epi_body(i, carry):
            run_all(ifft_unit(pl_last % 2, pl_last, i // 4, i % 4, True))
            return carry
        jax.lax.fori_loop(0, NI, epi_body, 0)

        def tile8(v):
            parts = [v[:, 128 * dt:128 * (dt + 1)] for dt in range(4)]
            return jnp.concatenate(parts + parts, axis=0)
        gam = g_ref[...].astype(jnp.float32)
        bet = b_ref[...].astype(jnp.float32)
        scs, shs = [], []
        for b in range(2):
            s1 = jnp.concatenate([jnp.sum(st[dt * 4 + 2 * b], axis=0, keepdims=True) for dt in range(4)], axis=1)
            s2 = jnp.concatenate([jnp.sum(st[dt * 4 + 2 * b + 1], axis=0, keepdims=True) for dt in range(4)], axis=1)
            mu = s1 * np.float32(1.0 / L)
            var = jnp.maximum(s2 * np.float32(1.0 / L) - mu * mu, 0.0)
            inv = np.float32(1.0 / (2 * N))
            sc = jax.lax.rsqrt(var * (inv * inv) + 1e-5) * (gam * inv)
            sh = bet - mu * sc
            scs.append(tile8(sc * 0.5)); shs.append(tile8(sh * 0.5))

        OROWS = 8 * L
        nblk = (OROWS + OB - 1) // OB

        def norm_rows(r0, nrows):
            q0 = r0 // 2 if isinstance(r0, int) else pl.multiple_of(r0 // 2, 8)
            u = hb32[pl.ds(q0, nrows // 2), :]
            u3 = u.reshape(nrows // 16, 8, 128)
            h0 = pltpu.bitcast(u3 << 16, jnp.float32)
            h1 = pltpu.bitcast(u3 & hmask, jnp.float32)
            y0 = _gelu_half(h0 * scs[0][None] + shs[0][None])
            y1 = _gelu_half(h1 * scs[1][None] + shs[1][None])
            pk = pltpu.pack_elementwise([y0, y1], packed_dtype=jnp.bfloat16).reshape(nrows // 2, 128)
            hb32[pl.ds(q0, nrows // 2), :] = pltpu.bitcast(pk, jnp.uint32)

        copies = []
        for blk in range(nblk):
            r0 = blk * OB
            n = min(OB, OROWS - r0)
            npad = ((n + 15) // 16) * 16
            SUB = 256

            def nb(i, carry, r0=r0):
                norm_rows(r0 + i * SUB, SUB)
                return carry
            if npad // SUB:
                jax.lax.fori_loop(0, npad // SUB, nb, 0)
            if npad % SUB:
                norm_rows(r0 + (npad // SUB) * SUB, npad % SUB)
            cp = pltpu.make_async_copy(hb.at[pl.ds(r0, n), :], o_hbm.at[pl.ds(r0, n), :], osem.at[blk])
            cp.start()
            copies.append(cp)
        for cp in copies:
            cp.wait()

    OROWS = 8 * L
    nblk = (OROWS + OB - 1) // OB
    out = pl.pallas_call(
        kernel,
        in_specs=[
            pl.BlockSpec(memory_space=pltpu.SMEM),
            pl.BlockSpec(memory_space=pl.ANY),
            pl.BlockSpec(memory_space=pl.ANY),
            pl.BlockSpec(memory_space=pltpu.VMEM),
            pl.BlockSpec(memory_space=pltpu.VMEM),
        ],
        out_specs=pl.BlockSpec(memory_space=pl.ANY),
        out_shape=jax.ShapeDtypeStruct((OROWS, 128), jnp.bfloat16),
        scratch_shapes=[
            pltpu.VMEM((60, D, 128), jnp.uint32),
pltpu.VMEM((60, D, 128), jnp.uint32),
pltpu.VMEM((60, D, 128), jnp.uint32),
pltpu.VMEM((60, D, 128), jnp.uint32),
            pltpu.VMEM((60, TC // 2, 2 * D), jnp.uint32),
            pltpu.VMEM((60, TC // 2, 2 * D), jnp.uint32),
            pltpu.VMEM((N * 4 * TC, 128), jnp.float32),
            pltpu.VMEM((N * 4 * TC, 128), jnp.float32),
            pltpu.VMEM((8 * XB, 128), jnp.uint32),
            pltpu.VMEM((HROWS // 2, 128), jnp.uint32),
            pltpu.VMEM((16, 8, 128), jnp.float32),
            pltpu.VMEM((160, 8, 128), jnp.float32),
            pltpu.VMEM((160, 8, 128), jnp.float32),
            pltpu.VMEM((80, 8, 128), jnp.float32),
            pltpu.VMEM((80, 8, 128), jnp.float32),
            pltpu.SemaphoreType.DMA((8,)),
            pltpu.SemaphoreType.DMA((4,)),
            pltpu.SemaphoreType.DMA((nblk,)),
        ],
        compiler_params=pltpu.CompilerParams(vmem_limit_bytes=126 * 1024 * 1024),
    )(jnp.zeros((2,), jnp.int32), x, w.reshape(K * D, D), gn_gamma.reshape(1, D), gn_beta.reshape(1, D))
    return out.reshape(L, 4, 2, 128).transpose(2, 0, 1, 3).reshape(B, L, D)
```

```python
import math
import numpy as np
import jax
import jax.numpy as jnp
import jax.experimental.pallas as pl
import jax.experimental.pallas.tpu as pltpu

N = 40
M = 25
C1 = math.cos(2 * math.pi / 5); C2 = math.cos(4 * math.pi / 5)
S1 = math.sin(2 * math.pi / 5); S2 = math.sin(4 * math.pi / 5)
R2 = math.sqrt(0.5)


class V:
    __slots__ = ("val", "neg")

    def __init__(self, val, neg=False):
        self.val = val
        self.neg = neg

    def get(self):
        return -self.val if self.neg else self.val


ZERO = V(None)


def vneg(a):
    return V(a.val, not a.neg)


def vadd(a, b):
    if a.val is None:
        return b
    if b.val is None:
        return a
    if a.neg == b.neg:
        return V(a.val + b.val, a.neg)
    if b.neg:
        return V(a.val - b.val, False)
    return V(b.val - a.val, False)


def vsub(a, b):
    return vadd(a, vneg(b))


def vmul(c, a):
    if a.val is None:
        return a
    return V(a.val * np.float32(-c if a.neg else c), False)


def cadd(a, b): return (vadd(a[0], b[0]), vadd(a[1], b[1]))
def csub(a, b): return (vsub(a[0], b[0]), vsub(a[1], b[1]))
def cmulr(c, a): return (vmul(c, a[0]), vmul(c, a[1]))


def cadd_i(a, b, s):
    if s > 0:
        return (vsub(a[0], b[1]), vadd(a[1], b[0]))
    return (vadd(a[0], b[1]), vsub(a[1], b[0]))


def dft5(x, s):
    t1 = cadd(x[1], x[4]); t2 = cadd(x[2], x[3]); t3 = csub(x[1], x[4]); t4 = csub(x[2], x[3])
    t5 = cadd(t1, t2)
    X0 = cadd(x[0], t5)
    a0 = cadd(x[0], cmulr((C1 + C2) / 2, t5))
    m2 = cmulr((C1 - C2) / 2, csub(t1, t2))
    a1 = cadd(a0, m2); a2 = csub(a0, m2)
    b1 = cadd(cmulr(S1, t3), cmulr(S2, t4))
    b2 = csub(cmulr(S2, t3), cmulr(S1, t4))
    return [X0, cadd_i(a1, b1, s), cadd_i(a2, b2, s), cadd_i(a2, b2, -s), cadd_i(a1, b1, -s)]


def dft4(x, s):
    a = cadd(x[0], x[2]); b = csub(x[0], x[2]); c = cadd(x[1], x[3]); d = csub(x[1], x[3])
    return [cadd(a, c), cadd_i(b, d, s), csub(a, c), cadd_i(b, d, -s)]


def dft8(x, s):
    E = dft4(x[0::2], s); O = dft4(x[1::2], s)
    o1 = O[1]; o3 = O[3]
    if s > 0:
        t1 = (vmul(R2, vsub(o1[0], o1[1])), vmul(R2, vadd(o1[0], o1[1])))
        t3 = (vmul(-R2, vadd(o3[0], o3[1])), vmul(R2, vsub(o3[0], o3[1])))
    else:
        t1 = (vmul(R2, vadd(o1[0], o1[1])), vmul(R2, vsub(o1[1], o1[0])))
        t3 = (vmul(R2, vsub(o3[1], o3[0])), vmul(-R2, vadd(o3[0], o3[1])))
    out = [None] * 8
    out[0] = cadd(E[0], O[0]); out[4] = csub(E[0], O[0])
    out[1] = cadd(E[1], t1); out[5] = csub(E[1], t1)
    out[2] = cadd_i(E[2], O[2], s); out[6] = cadd_i(E[2], O[2], -s)
    out[3] = cadd(E[3], t3); out[7] = csub(E[3], t3)
    return out


def crt(k1, k2):
    return [k for k in range(N) if k % 5 == k1 and k % 8 == k2][0]


def _gelu(h):
    c = 0.7978845608028654
    inner = h * (np.float32(c) + np.float32(c * 0.044715) * (h * h))
    return (np.float32(0.5) * h) * (np.float32(1.0) + jnp.tanh(inner))


def _gelu_half(u):
    c = 0.7978845608028654
    z = u * (np.float32(2 * c) + np.float32(8 * c * 0.044715) * (u * u))
    return u + u * jnp.tanh(z)


@jax.jit
def pallas_standalone__self_sup_conv_stem_wavlm__speech_kernel(
    x: jax.Array,
    w: jax.Array,
    gn_gamma: jax.Array,
    gn_beta: jax.Array,
):
    B, T, D = x.shape
    K = w.shape[0]
    L = (T - K) // 2 + 1
    assert (B, T, D, K) == (2, 16000, 512, 31)
    U = T // 2
    G = 5
    TC = 2 * 8 * G
    NCH = U // (M * 8 * G)
    CU = M * 8 * G
    XR = 2032
    XB = 2064
    NI = 20
    OB = 2048
    HROWS = 8 * U
    UNROLL = 4
    KSPLIT = 4
    LAG_MAIN = 0
    LAG_ST = 0
    FFT_WEIGHT = 16 * 54 + 5 * 152
    NG = 1

    def kernel(flag_ref, x_hbm, w_hbm, g_ref, b_ref, o_hbm, wh0, wh1, wh2, wh3, xh0, xh1, yh0, yh1, xs, hb, st, tF0, tF1, tI0, tI1, xsem, wsem, osem):
        whs = [wh0, wh1, wh2, wh3]
        tF = [tF0, tF1]
        tI = [tI0, tI1]
        dz = flag_ref[0]
        dz2 = flag_ref[1]
        xh = [xh0, xh1]
        yh = [yh0, yh1]
        xs32 = xs
        hb32 = hb
        xs = xs32.bitcast(jnp.bfloat16)
        hb = hb32.bitcast(jnp.bfloat16)
        hmask = np.uint32(0xFFFF0000)

        def x_copies(c, slot, dts=(0, 1, 2, 3)):
            start = pl.multiple_of(jnp.minimum(c * (2 * CU), T - XR), 16)
            return [pltpu.make_async_copy(
                x_hbm.at[b, pl.ds(start, XR), pl.ds(128 * dt, 128)],
                xs.at[pl.ds(pl.multiple_of(((slot * 2 + b) * 4 + dt) * XB, 16), XR), :], xsem.at[slot * 4 + dt])
                for dt in dts for b in range(2)]

        def w_copies(dt):
            return [pltpu.make_async_copy(
                w_hbm.at[:, pl.ds(128 * dt, 128)],
                hb.at[pl.ds(dt * K * D, K * D), :], wsem.at[dt])]

        for cp in x_copies(0, 0):
            cp.start()

        for i in range(16):
            xs32[(i * XB + XR) // 2:(i + 1) * XB // 2, :] = jnp.zeros(((XB - XR) // 2, 128), jnp.uint32)
        for slot in range(2):
            xh[slot][0] = jnp.zeros((TC // 2, 2 * D), jnp.uint32)
        st[...] = jnp.zeros(st.shape, jnp.float32)

        TOK = [None]
        HIST = []
        TOKS = []
        LAGV = [LAG_MAIN]
        never_s = [flag_ref[0] > 0]

        def gate(v):
            if TOK[0] is None:
                return v
            HIST.append(TOK[0])
            t = TOKS[max(0, len(TOKS) - 1 - LAGV[0])]
            if v.dtype != t.dtype:
                t = pltpu.bitcast(t, v.dtype)
            return jnp.where(never_s[0], t, v)

        def gateV(a):
            return V(gate(a.val), a.neg)

        def stash(ref, idx, cv):
            out = []
            for c_, v in enumerate(cv):
                if v.val is None:
                    out.append(None)
                else:
                    ref[dz + 2 * idx + c_] = v.val
                    out.append(v.neg)
            return out

        def fetch(ref, idx, negs):
            return tuple(ZERO if ng is None else V(ref[dz2 + 2 * idx + c_], ng) for c_, ng in enumerate(negs))

        def fft_unit(slot, off, g, dt, tr=0):
            base = (slot * 8 + dt) * (XB // 2) + off + g * (8 * M)
            lane0 = pl.multiple_of(dt * 128, 128)
            lane1 = pl.multiple_of(dt * 128 + D, 128)
            row0 = pl.multiple_of(g * 8, 8)
            T1 = []
            for b in range(2):
                Tb = []
                for p2 in range(8):
                    zin = []
                    for p1 in range(5):
                        p = (8 * p1 + 5 * p2) % N
                        u = xs32[pl.ds(base + b * (2 * XB) + p, 8, stride=M), :]
                        if p1 < NG:
                            u = gate(u)
                        zin.append((V(pltpu.bitcast(u << 16, jnp.float32)),
                                    V(pltpu.bitcast(u & hmask, jnp.float32))))
                    o5 = dft5(zin, -1)
                    Tb.append([stash(tF[tr], (b * 8 + p2) * 5 + k1, o5[k1]) for k1 in range(5)])
                    yield 54
                T1.append(Tb)

            def emit(m, lane, va, vb):
                v = pltpu.pack_elementwise([va.get(), vb.get()], packed_dtype=jnp.bfloat16)
                xh[slot][m, pl.ds(row0, 8), pl.ds(lane, 128)] = pltpu.bitcast(v, jnp.uint32)

            for k1 in range(5):
                r = []
                for b in range(2):
                    zz = [fetch(tF[tr], (b * 8 + p2) * 5 + k1, T1[b][p2][k1]) for p2 in range(8)]
                    zz[0] = (gateV(zz[0][0]), zz[0][1])
                    r.append(dft8(zz, -1))
                    yield 56
                for k2 in range(8):
                    k = crt(k1, k2)
                    (a0, b0), (a1, b1) = r[0][k2], r[1][k2]
                    if k == 0:
                        emit(2, lane0, a0, a1); emit(2, lane1, b0, b1)
                    elif k == 20:
                        emit(1, lane0, a0, a1); emit(1, lane1, b0, b1)
                    elif k < 20:
                        emit(3 * k, lane0, vadd(a0, b0), vadd(a1, b1))
                        emit(3 * k + 1, lane0, a0, a1)
                        emit(3 * k + 2, lane0, b0, b1)
                    else:
                        kk = N - k
                        emit(3 * kk, lane1, vsub(a0, b0), vsub(a1, b1))
                        emit(3 * kk + 1, lane1, a0, a1)
                        emit(3 * kk + 2, lane1, b0, b1)
                yield 40

        def w_unit(dt, rb, tr=0):
            T1 = []
            raw = {}

            def getraw(j):
                if j not in raw:
                    raw[j] = hb32[pl.ds(pl.multiple_of((dt * K + j) * (D // 2) + rb * 8, 8), 8), :]
                return raw[j]
            for h in range(2):
                def ld(j, gt=False):
                    if j >= K:
                        return ZERO
                    u = getraw(j)
                    if gt:
                        u = gate(u)
                    return V(pltpu.bitcast((u << 16) if h == 0 else (u & hmask), jnp.float32))
                Tb = []
                for p2 in range(8):
                    zin = []
                    first = True
                    for p1 in range(5):
                        p = (8 * p1 + 5 * p2) % N
                        if p < 16:
                            zin.append((ld(2 * p, first), vneg(ld(2 * p + 1))))
                            first = False
                        else:
                            zin.append((ZERO, ZERO))
                    o5 = dft5(zin, +1)
                    Tb.append([stash(tF[tr], (h * 8 + p2) * 5 + k1, o5[k1]) for k1 in range(5)])
                    yield 32
                T1.append(Tb)

            def emit(m, half, va, vb):
                v = pltpu.pack_elementwise([va.get(), vb.get()], packed_dtype=jnp.bfloat16)
                whs[dt][m, pl.ds(pl.multiple_of(half * (D // 2) + rb * 8, 8), 8), :] = pltpu.bitcast(v, jnp.uint32)

            for k1 in range(5):
                r = []
                for h in range(2):
                    zz = [fetch(tF[tr], (h * 8 + p2) * 5 + k1, T1[h][p2][k1]) for p2 in range(8)]
                    zz[0] = (gateV(zz[0][0]), zz[0][1])
                    r.append(dft8(zz, +1))
                    yield 56
                for k2 in range(8):
                    k = crt(k1, k2)
                    q = [r[0][k2], r[1][k2]]
                    if k == 0:
                        emit(2, 0, *[vmul(-2.0, a[0]) for a in q])
                        emit(2, 1, *[vmul(2.0, a[1]) for a in q])
                    elif k == 20:
                        emit(1, 0, *[vmul(2.0, a[0]) for a in q])
                        emit(1, 1, *[vmul(-2.0, a[1]) for a in q])
                    elif k < 20:
                        emit(3 * k, 0, *[a[0] for a in q])
                        emit(3 * k + 1, 0, *[vsub(a[1], a[0]) for a in q])
                        emit(3 * k + 2, 0, *[vadd(a[0], a[1]) for a in q])
                    else:
                        kk = N - k
                        emit(3 * kk, 1, *[a[0] for a in q])
                        emit(3 * kk + 1, 1, *[vneg(vadd(a[0], a[1])) for a in q])
                        emit(3 * kk + 2, 1, *[vsub(a[1], a[0]) for a in q])
                yield 66
        W_WEIGHT = 16 * 32 + 5 * (112 + 66)

        def chain(gens):
            for g_ in gens:
                yield from g_

        def mm_piece(slot, kap, dt):
            ks = []
            for j in range(3):
                acc = None
                for kh in range(KSPLIT):
                    kw = 2 * D // KSPLIT
                    a = pltpu.bitcast(xh[slot][3 * kap + j, :, kh * kw:(kh + 1) * kw], jnp.bfloat16)
                    mw = jnp.maximum(3 * kap, 1) if j == 0 else 3 * kap + j
                    bb = pltpu.bitcast(whs[dt][mw, kh * kw // 2:(kh + 1) * kw // 2, :], jnp.bfloat16)
                    d = jnp.dot(a, bb, preferred_element_type=jnp.float32)
                    acc = d if acc is None else acc + d
                    TOK[0] = d[0:8, :]
                    TOKS.append(TOK[0])
                    yield 1
                ks.append(acc)
            r0 = pl.multiple_of((2 * kap * 4 + dt) * TC, 8)
            r1 = pl.multiple_of(((2 * kap + 1) * 4 + dt) * TC, 8)
            yh[slot][pl.ds(r0, TC), :] = ks[0] - ks[2]
            yh[slot][pl.ds(r1, TC), :] = ks[0] + ks[1]

        def mm_unit(slot, kap):
            for dt in range(4):
                yield from mm_piece(slot, kap, dt)

        def run_all(gen):
            for _ in gen:
                pass

        def interleave(mm, others, npieces):
            tot = sum(w for _, w in others)
            done = [0.0] * len(others)
            alive = [True] * len(others)
            i = 0
            for _ in mm:
                i += 1
                target = tot * min(i, npieces) / npieces
                while sum(done) < target and any(alive):
                    k = min((k for k in range(len(others)) if alive[k]), key=lambda k: done[k] / others[k][1])
                    try:
                        done[k] += next(others[k][0])
                    except StopIteration:
                        alive[k] = False
            for gen, _ in others:
                run_all(gen)

        def ifft_unit(slot, c, g, dt, masked, tr=0):
            rowa = dt * TC + g * 16
            rowb = rowa + 1

            def ld(v, row):
                return V(yh[slot][pl.ds(v * (4 * TC) + row, 8, stride=2), :])
            Dk = [None] * N
            Dk[0] = (ld(0, rowa), ld(0, rowb))
            Dk[20] = (ld(1, rowa), ld(1, rowb))
            for k in range(1, 20):
                ar, ai = ld(2 * k, rowa), ld(2 * k + 1, rowa)
                br, bi = ld(2 * k, rowb), ld(2 * k + 1, rowb)
                Dk[k] = (vsub(ar, bi), vadd(ai, br))
                Dk[N - k] = (vadd(ar, bi), vsub(br, ai))
            T1 = [None] * 8
            for p2 in (0, 1, 7, 2, 6, 3, 5, 4):
                o5 = dft5([(gateV(Dk[(8 * p1 + 5 * p2) % N][0]), Dk[(8 * p1 + 5 * p2) % N][1]) if p1 < NG else Dk[(8 * p1 + 5 * p2) % N] for p1 in range(5)], +1)
                T1[p2] = [stash(tI[tr], p2 * 5 + k1, o5[k1]) for k1 in range(5)]
                yield 54
            t0 = c * (8 * G) + g * 8
            hrow = t0 * (4 * M) + dt
            s = [None] * 4
            if masked:
                lrow = (t0 + jax.lax.broadcasted_iota(jnp.int32, (8, 128), 0)) * M
            for k1 in range(5):
                zz = [fetch(tI[tr], p2 * 5 + k1, T1[p2][k1]) for p2 in range(8)]
                zz[0] = (gateV(zz[0][0]), zz[0][1])
                r = dft8(zz, +1)
                for k2 in range(8):
                    n = crt(k1, k2)
                    if n >= M:
                        continue
                    h0, h1 = r[k2][0].get(), r[k2][1].get()
                    if masked:
                        ok = lrow < (L - n)
                        h0 = jnp.where(ok, h0, 0.0)
                        h1 = jnp.where(ok, h1, 0.0)
                    for i, hv in enumerate((h0, h1)):
                        sq = hv * hv
                        s[2 * i] = hv if s[2 * i] is None else s[2 * i] + hv
                        s[2 * i + 1] = sq if s[2 * i + 1] is None else s[2 * i + 1] + sq
                    pk = pltpu.pack_elementwise([h0, h1], packed_dtype=jnp.bfloat16)
                    hb32[pl.ds(hrow + 4 * n, 8, stride=4 * M), :] = pltpu.bitcast(pk, jnp.uint32)
                yield 90
            for i in range(4):
                idx = dt * 4 + i
                st[idx] = st[idx] + s[i]

        def pro_body(i, carry):
            dt = i // G

            @pl.when(i % G == 0)
            def _():
                for b in range(2):
                    pltpu.make_async_copy(
                        x_hbm.at[b, pl.ds(0, XR), pl.ds(0, 128)],
                        xs.at[pl.ds(0, XR), :], xsem.at[dt]).wait()

            @pl.when(i == 0)
            def _():
                for cp in w_copies(0):
                    cp.start()

            run_all(fft_unit(0, 0, i % G, dt))
            return carry
        jax.lax.fori_loop(0, NI, pro_body, 0)

        for cp in w_copies(0):
            cp.wait()

        def w_body(rb, carry):
            run_all(w_unit(0, rb))
            return carry
        for cp in w_copies(1):
            cp.start()
        jax.lax.fori_loop(0, D // 16, w_body, 0)

        def stage(dt):
            for cp in w_copies(dt + 1):
                cp.wait()
            if dt < 2:
                for cp in w_copies(dt + 2):
                    cp.start()
            if dt == 1:
                for cp in x_copies(1, 1):
                    cp.start()

            def body(it, carry):
                mm = chain([mm_piece(0, it * 5 + u, dt) for u in range(5)])
                others = [(chain([w_unit(dt + 1, it * 8 + u, u % 2) for u in range(8)]), 8 * W_WEIGHT)]
                interleave(mm, others, 15 * KSPLIT)
                TOK[0] = None; TOKS.clear()
                return carry
            jax.lax.fori_loop(0, 4, body, 0)
        LAGV[0] = LAG_ST
        for dt_ in range(3):
            stage(dt_)

        for cp in x_copies(1, 1):
            cp.wait()
        for cp in x_copies(2, 0):
            cp.start()

        def stage3_body(it, carry):
            mm = chain([mm_piece(0, it * 5 + u, 3) for u in range(5)])
            others = [(chain([fft_unit(1, 0, (it * 5 + u) // 4, (it * 5 + u) % 4, u % 2) for u in range(5)]), 5 * FFT_WEIGHT)]
            interleave(mm, others, 15 * KSPLIT)
            TOK[0] = None; TOKS.clear()
            return carry
        jax.lax.fori_loop(0, 4, stage3_body, 0)

        LAGV[0] = LAG_MAIN
        def phase(p, cur, do_fft=True):
            nxt = 1 - cur
            if do_fft:
                for cp in x_copies(p + 1, nxt):
                    cp.wait()

                @pl.when(p + 2 < NCH)
                def _():
                    for cp in x_copies(p + 2, cur):
                        cp.start()
            off = jnp.where(p + 1 >= NCH - 1, (XR - 2 * CU) // 2, 0)
            cprev = p - 1

            def body(i, carry):
                for u in range(UNROLL):
                    ii = i * UNROLL + u
                    others = [(ifft_unit(nxt, cprev, ii // 4, ii % 4, False, u % 2), 8 * 54 + 5 * 90)]
                    if do_fft:
                        others.append((fft_unit(nxt, off, ii // 4, ii % 4, u % 2), FFT_WEIGHT))
                    interleave(mm_unit(cur, ii), others, 12 * KSPLIT)
                    TOK[0] = None; TOKS.clear()
                return carry
            jax.lax.fori_loop(0, NI // UNROLL, body, 0)

        def phase2(q, carry):
            phase(2 * q + 1, 1)
            phase(2 * q + 2, 0)
            return carry
        jax.lax.fori_loop(0, NCH // 2 - 1, phase2, 0)
        pl_last = NCH - 1

        def last_stage(dt):
            def body(it, carry):
                mm = chain([mm_piece(1, it * 4 + u, dt) for u in range(4)])
                others = [(ifft_unit(0, pl_last - 1, it, dt, False, 0), 8 * 54 + 5 * 90)]
                if dt > 0:
                    others.append((ifft_unit(1, pl_last, it, dt - 1, True, 1), 8 * 54 + 5 * 90))
                interleave(mm, others, 12 * KSPLIT)
                TOK[0] = None; TOKS.clear()
                return carry
            jax.lax.fori_loop(0, G, body, 0)
        for dt_ in range(4):
            last_stage(dt_)

        def epi_body(i, carry):
            run_all(ifft_unit(1, pl_last, i, 3, True))
            return carry
        jax.lax.fori_loop(0, G, epi_body, 0)

        def tile8(v):
            parts = [v[:, 128 * dt:128 * (dt + 1)] for dt in range(4)]
            return jnp.concatenate(parts + parts, axis=0)
        gam = g_ref[...].astype(jnp.float32)
        bet = b_ref[...].astype(jnp.float32)
        scs, shs = [], []
        for b in range(2):
            s1 = jnp.concatenate([jnp.sum(st[dt * 4 + 2 * b], axis=0, keepdims=True) for dt in range(4)], axis=1)
            s2 = jnp.concatenate([jnp.sum(st[dt * 4 + 2 * b + 1], axis=0, keepdims=True) for dt in range(4)], axis=1)
            mu = s1 * np.float32(1.0 / L)
            var = jnp.maximum(s2 * np.float32(1.0 / L) - mu * mu, 0.0)
            inv = np.float32(1.0 / (2 * N))
            sc = jax.lax.rsqrt(var * (inv * inv) + 1e-5) * (gam * inv)
            sh = bet - mu * sc
            scs.append(tile8(sc * 0.5)); shs.append(tile8(sh * 0.5))

        OROWS = 8 * L
        nblk = (OROWS + OB - 1) // OB

        def norm_rows(r0, nrows):
            q0 = r0 // 2 if isinstance(r0, int) else pl.multiple_of(r0 // 2, 8)
            u = hb32[pl.ds(q0, nrows // 2), :]
            u3 = u.reshape(nrows // 16, 8, 128)
            h0 = pltpu.bitcast(u3 << 16, jnp.float32)
            h1 = pltpu.bitcast(u3 & hmask, jnp.float32)
            y0 = _gelu_half(h0 * scs[0][None] + shs[0][None])
            y1 = _gelu_half(h1 * scs[1][None] + shs[1][None])
            pk = pltpu.pack_elementwise([y0, y1], packed_dtype=jnp.bfloat16).reshape(nrows // 2, 128)
            hb32[pl.ds(q0, nrows // 2), :] = pltpu.bitcast(pk, jnp.uint32)

        copies = []
        for blk in range(nblk):
            r0 = blk * OB
            n = min(OB, OROWS - r0)
            npad = ((n + 15) // 16) * 16
            SUB = 256

            def nb(i, carry, r0=r0):
                norm_rows(r0 + i * SUB, SUB)
                return carry
            if npad // SUB:
                jax.lax.fori_loop(0, npad // SUB, nb, 0)
            if npad % SUB:
                norm_rows(r0 + (npad // SUB) * SUB, npad % SUB)
            cp = pltpu.make_async_copy(hb.at[pl.ds(r0, n), :], o_hbm.at[pl.ds(r0, n), :], osem.at[blk])
            cp.start()
            copies.append(cp)
        for cp in copies:
            cp.wait()

    OROWS = 8 * L
    nblk = (OROWS + OB - 1) // OB
    out = pl.pallas_call(
        kernel,
        in_specs=[
            pl.BlockSpec(memory_space=pltpu.SMEM),
            pl.BlockSpec(memory_space=pl.ANY),
            pl.BlockSpec(memory_space=pl.ANY),
            pl.BlockSpec(memory_space=pltpu.VMEM),
            pl.BlockSpec(memory_space=pltpu.VMEM),
        ],
        out_specs=pl.BlockSpec(memory_space=pl.ANY),
        out_shape=jax.ShapeDtypeStruct((OROWS, 128), jnp.bfloat16),
        scratch_shapes=[
            pltpu.VMEM((60, D, 128), jnp.uint32),
pltpu.VMEM((60, D, 128), jnp.uint32),
pltpu.VMEM((60, D, 128), jnp.uint32),
pltpu.VMEM((60, D, 128), jnp.uint32),
            pltpu.VMEM((60, TC // 2, 2 * D), jnp.uint32),
            pltpu.VMEM((60, TC // 2, 2 * D), jnp.uint32),
            pltpu.VMEM((N * 4 * TC, 128), jnp.float32),
            pltpu.VMEM((N * 4 * TC, 128), jnp.float32),
            pltpu.VMEM((8 * XB, 128), jnp.uint32),
            pltpu.VMEM((HROWS // 2, 128), jnp.uint32),
            pltpu.VMEM((16, 8, 128), jnp.float32),
            pltpu.VMEM((160, 8, 128), jnp.float32),
            pltpu.VMEM((160, 8, 128), jnp.float32),
            pltpu.VMEM((80, 8, 128), jnp.float32),
            pltpu.VMEM((80, 8, 128), jnp.float32),
            pltpu.SemaphoreType.DMA((8,)),
            pltpu.SemaphoreType.DMA((4,)),
            pltpu.SemaphoreType.DMA((nblk,)),
        ],
        compiler_params=pltpu.CompilerParams(vmem_limit_bytes=126 * 1024 * 1024),
    )(jnp.zeros((2,), jnp.int32), x, w.reshape(K * D, D), gn_gamma.reshape(1, D), gn_beta.reshape(1, D))
    return out.reshape(L, 4, 2, 128).transpose(2, 0, 1, 3).reshape(B, L, D)
```
